```python
import os as _os
_os.environ.setdefault("JAX_PLATFORMS", "cpu")
import jax
import jax.numpy as jnp

def _softmax(x, axis=-1):
    return jax.nn.softmax(x, axis=axis)
def _gelu(x):
    return jax.nn.gelu(x, approximate=True)
def _silu(x):
    return jax.nn.silu(x)
def _sigmoid(x):
    return jax.nn.sigmoid(x)
def _layernorm(x, axis=-1, eps=1e-5):
    m = jnp.mean(x, axis=axis, keepdims=True)
    v = jnp.var(x, axis=axis, keepdims=True)
    return (x - m) / jnp.sqrt(v + eps)
def _scatter_add(tgt, idx, src, axis=0):
    return tgt.at[idx].add(src)
def _segment_sum(src, seg, n):
    return jax.ops.segment_sum(src, seg, n)
class _Rng:
    def __init__(self, key):
        self._k = key
    def _next(self):
        self._k, sub = jax.random.split(self._k)
        return sub
    def normal(self, shape):
        return jax.random.normal(self._next(), shape, dtype=jnp.bfloat16)
    def randint(self, lo, hi, shape):
        return jax.random.randint(self._next(), shape, lo, hi, dtype=jnp.int32)
    def uniform(self, shape, lo=0.0, hi=1.0):
        return jax.random.uniform(self._next(), shape, jnp.bfloat16, lo, hi)
    def permutation(self, n):
        return jax.random.permutation(self._next(), n)


kernel_name = 'concat_heads__sliding_local_dilated__sliding_block__prompt'

def setup_inputs():
    _rng = _Rng(jax.random.key(int.from_bytes(__import__("os").urandom(4), "little")))
    _w = (lambda a: (lambda t: t.astype(jnp.bfloat16) if jnp.issubdtype(t.dtype, jnp.floating) else t)(jnp.asarray(a)))
    def _A_setup():
        B, S, D = 1, 2048, 1024
        return {
            "x": _w((lambda *s: _rng.normal(s) * 0.2)(B, S, D)),
            "wqkv": _w((lambda *s: _rng.normal(s) * 0.2)(D, 3 * D)),
            "wo": _w((lambda *s: _rng.normal(s) * 0.05)(D, D)),
        }
    _A_in = _A_setup()

    def _B_setup():
        B, S, D = 1, 2048, 1024
        return {
            "x": _w((lambda *s: _rng.normal(s) * 0.2)(B, S, D)),
            "wqkv": _w((lambda *s: _rng.normal(s) * 0.2)(D, 3 * D)),
            "wo": _w((lambda *s: _rng.normal(s) * 0.05)(D, D)),
        }
    _B_in = _B_setup()

    return {
        "A_x": _A_in["x"],
        "A_wqkv": _A_in["wqkv"],
        "A_wo": _A_in["wo"],
        "B_x": _B_in["x"],
        "B_wqkv": _B_in["wqkv"],
        "B_wo": _B_in["wo"],
    }

def reference(A_x, A_wqkv, A_wo, B_x, B_wqkv, B_wo):
    def _A_ref(x, wqkv, wo):
        B, S, D = x.shape
        H = 32; Dh = D // H
        W, dil = 8, 2
        qkv = (lambda x, *d: x.transpose(*d))((x @ wqkv).reshape(B, S, 3, H, Dh), 2, 0, 3, 1, 4)
        q, k, v = qkv[0], qkv[1], qkv[2]
        scale = Dh ** -0.5
        pos = jnp.arange(S)
        off = jnp.arange(W) * dil
        idx = pos[:, None] - off[None, :]
        mask = idx >= 0
        idx_c = jnp.where(mask, idx, 0).reshape(-1)
        kg = k[:, :, idx_c, :].reshape(B, H, S, W, Dh)
        vg = v[:, :, idx_c, :].reshape(B, H, S, W, Dh)
        logits = jnp.einsum("bhsd,bhswd->bhsw", q, kg) * scale
        logits = jnp.where(mask[None, None, :, :], logits, -1e9)
        attn = _softmax(logits, axis=-1)
        o = jnp.einsum("bhsw,bhswd->bhsd", attn, vg)
        return (lambda x, *d: x.transpose(*d))(o, 0, 2, 1, 3).reshape(B, S, D) @ wo

    def _B_ref(x, wqkv, wo):
        B, S, D = x.shape
        H = 32; Dh = D // H; W = 256
        qkv = (lambda x, *d: x.transpose(*d))((x @ wqkv).reshape(B, S, 3, H, Dh), 2, 0, 3, 1, 4)
        q, k, v = qkv[0], qkv[1], qkv[2]
        scores = jnp.einsum("bhqd,bhkd->bhqk", q, k) * (Dh ** -0.5)
        idx = jnp.arange(S)
        mask = (idx[:, None] - idx[None, :] >= 0) & (idx[:, None] - idx[None, :] < W)
        scores = jnp.where(mask[None, None], scores, -1e9)
        p = _softmax(scores, axis=-1)
        o = jnp.einsum("bhqk,bhkd->bhqd", p, v)
        return (lambda x, *d: x.transpose(*d))(o, 0, 2, 1, 3).reshape(B, S, D) @ wo

    a = _A_ref(A_x, A_wqkv, A_wo)
    b = _B_ref(B_x, B_wqkv, B_wo)
    return jnp.concatenate([a, b], axis=-1)
```

```python
import jax
import jax.numpy as jnp
from jax import lax
import jax.experimental.pallas as pl
import jax.experimental.pallas.tpu as pltpu

S, D, H, DH = 2048, 1024, 32, 32
TS = 256
NB = S // TS
QB = 128
WB = 256
WA, DIL = 8, 2
PADA = 16
RC = 64
NEG = -1e9
LOG2E = 1.4426950408889634
QSCALE = (DH ** -0.5) * LOG2E
NCHUNK = 512
NQKV = 3 * D // NCHUNK
NO = D // NCHUNK
FB = 128


def _kernel(xa_ref, xb_ref, wqkva_hbm, woa_hbm, wqkvb_hbm, wob_hbm, out_ref,
            wqkva, woa, wqkvb, wob, qa_s, ka_s, va_s, qb_s, kb_s, vb_s, oa_s, ob_s, xp_s, xpa_s, sems):
    step = pl.program_id(0)
    f32, bf16 = jnp.float32, jnp.bfloat16

    copies = []
    sid = 0
    for src, dst, n in ((wqkva_hbm, wqkva, NQKV), (woa_hbm, woa, NO),
                        (wqkvb_hbm, wqkvb, NQKV), (wob_hbm, wob, NO)):
        lst = []
        for c in range(n):
            cs = pl.ds(c * NCHUNK, NCHUNK)
            lst.append(pltpu.make_async_copy(src.at[:, cs], dst.at[:, cs], sems.at[sid]))
            sid += 1
        copies.append(lst)

    row0 = pl.multiple_of(step * TS, TS)
    row0h = pl.multiple_of(step * (TS // 2), TS // 2)

    first = step == 0

    @pl.when(first)
    def _():
        for lst in copies:
            for cp in lst:
                cp.start()
        ka_s[:, pl.ds(0, PADA), :] = jnp.zeros((8, PADA, 128), f32)
        va_s[:, pl.ds(0, PADA), :] = jnp.zeros((8, PADA, 128), f32)
        kb_s[pl.ds(0, WB // 2), :] = jnp.zeros((WB // 2, D), jnp.uint32)
        vb_s[:, pl.ds(0, WB)] = jnp.zeros((D // 2, WB), jnp.uint32)
        for cp in copies[0]:
            cp.wait()

    def body():
        def wait(cp):
            @pl.when(first)
            def _():
                cp.wait()

        def qkv_a(c):
            xa = pltpu.bitcast(xpa_s[...], bf16)
            r = jnp.dot(xa, wqkva[:, c * NCHUNK:(c + 1) * NCHUNK], preferred_element_type=f32)
            r = r.astype(bf16).astype(f32)
            which, col = divmod(c * NCHUNK, D)
            if which == 0:
                qa_s[:, col:col + NCHUNK] = r * QSCALE
            else:
                dst = ka_s if which == 1 else va_s
                for j in range(NCHUNK // 128):
                    dst[col // 128 + j, pl.ds(row0 + PADA, TS), :] = r[:, j * 128:(j + 1) * 128]

        li = lax.broadcasted_iota(jnp.int32, (128, 128), 0) // DH
        lj = lax.broadcasted_iota(jnp.int32, (128, 128), 1) // DH
        bd = jnp.where(li == lj, 1.0, 0.0).astype(bf16)

        def a_unit(rc, g):
            lanes = slice(g * 128, (g + 1) * 128)
            r_loc = rc * RC
            q = qa_s[r_loc:r_loc + RC, lanes]
            base = pl.multiple_of(row0 + r_loc, RC)
            kwin = ka_s.at[g, pl.ds(base, RC + PADA), :]
            vwin = va_s.at[g, pl.ds(base, RC + PADA), :]
            prods = []
            for w in range(WA):
                kw = kwin[PADA - DIL * w:PADA - DIL * w + RC, :]
                prods.append(q * kw)
            lg = jnp.dot(jnp.concatenate(prods, axis=0).astype(bf16), bd, preferred_element_type=f32)
            ls = [lg[w * RC:(w + 1) * RC] for w in range(WA)]
            if rc == 0:
                pos = row0 + lax.broadcasted_iota(jnp.int32, (RC, 128), 0)
                ls = [ls[0]] + [jnp.where(pos >= DIL * w, ls[w], NEG) for w in range(1, WA)]
            m = ls[0]
            for w in range(1, WA):
                m = jnp.maximum(m, ls[w])
            den = None
            acc = None
            for w in range(WA):
                p = jnp.exp2(ls[w] - m)
                pv = p * vwin[PADA - DIL * w:PADA - DIL * w + RC, :]
                den = p if den is None else den + p
                acc = pv if acc is None else acc + pv
            oa_s[r_loc // 2:(r_loc + RC) // 2, lanes] = pltpu.bitcast((acc * pl.reciprocal(den, approx=True)).astype(bf16), jnp.uint32)

        def out_a(c, wd):
            r = jnp.dot(pltpu.bitcast(oa_s[...], bf16), woa[:, c * wd:(c + 1) * wd], preferred_element_type=f32)
            out_ref[:, c * wd:(c + 1) * wd] = r.astype(bf16)

        def qkv_b(c, wd):
            xb = pltpu.bitcast(xp_s[...], bf16)
            r = jnp.dot(xb, wqkvb[:, c * wd:(c + 1) * wd], preferred_element_type=f32)
            which, col = divmod(c * wd, D)
            if which == 0:
                qb_s[:, col:col + wd] = pltpu.bitcast((r * QSCALE).astype(bf16), jnp.uint32)
            elif which == 1:
                kb_s[pl.ds(row0h + WB // 2, TS // 2), col:col + wd] = pltpu.bitcast(r.astype(bf16), jnp.uint32)
            else:
                vb_s[col // 2:(col + wd) // 2, pl.ds(row0 + WB, TS)] = pltpu.bitcast(r.T.astype(bf16), jnp.uint32)

        lane_head = lax.broadcasted_iota(jnp.int32, (QB, 128), 1) // DH
        b_idx = lax.broadcasted_iota(jnp.int32, (QB, 4 * QB), 0)
        a_idx = lax.broadcasted_iota(jnp.int32, (QB, 4 * QB), 1) % QB
        causal = b_idx <= a_idx

        def b_qk(qi, g):
            lanes = slice(g * 128, (g + 1) * 128)
            r_loc = qi * QB
            r_globh = pl.multiple_of(row0h + r_loc // 2, QB // 2)
            q4 = pltpu.bitcast(qb_s[r_loc // 2:(r_loc + QB) // 2, lanes], bf16)
            qs = jnp.concatenate(
                [jnp.where(lane_head == h, q4, jnp.zeros_like(q4)) for h in range(4)], axis=0)
            k4 = pltpu.bitcast(kb_s[pl.ds(r_globh, 3 * QB // 2), lanes], bf16)
            return lax.dot_general(k4, qs, (((1,), (1,)), ((), ())), preferred_element_type=f32)

        def b_rest(qi, g, s):
            lanes = slice(g * 128, (g + 1) * 128)
            r_loc = qi * QB
            r_glob = pl.multiple_of(row0 + r_loc, QB)
            s0, s1, s2 = s[0:QB], s[QB:2 * QB], s[2 * QB:3 * QB]
            s0 = jnp.where(first, NEG, s0)
            if qi == 0:
                s1 = jnp.where(first, NEG, s1)
            s02 = jnp.where(causal, s2, s0)
            m = jnp.max(jnp.maximum(s02, s1), axis=0, keepdims=True)
            p02 = jnp.exp2(s02 - m)
            p1 = jnp.exp2(s1 - m)
            l = jnp.sum(p02 + p1, axis=0, keepdims=True)
            p0 = jnp.where(causal, 0.0, p02)
            p2 = jnp.where(causal, p02, 0.0)
            inv = pl.reciprocal(l, approx=True)
            ots = []
            for h in range(4):
                f0 = g * 128 + h * DH
                vt = pltpu.bitcast(vb_s[f0 // 2:(f0 + DH) // 2, pl.ds(r_glob, 3 * QB)], bf16)
                hs = slice(h * QB, (h + 1) * QB)
                ph = jnp.concatenate([p0[:, hs], p1[:, hs], p2[:, hs]], axis=0).astype(bf16)
                ot = jnp.dot(vt, ph, preferred_element_type=f32)
                ots.append(ot * inv[:, h * QB:(h + 1) * QB])
            o4 = jnp.concatenate(ots, axis=0).T
            ob_s[r_loc // 2:(r_loc + QB) // 2, lanes] = pltpu.bitcast(o4.astype(bf16), jnp.uint32)

        def out_b(qi, c, wd):
            r = jnp.dot(pltpu.bitcast(ob_s[qi * QB // 2:(qi + 1) * QB // 2, :], bf16),
                        wob[:, c * wd:(c + 1) * wd], preferred_element_type=f32)
            out_ref[qi * QB:(qi + 1) * QB, D + c * wd:D + (c + 1) * wd] = r.astype(bf16)

        xpa_s[...] = pltpu.bitcast(xa_ref[...], jnp.uint32)
        for c in range(NQKV):
            qkv_a(c)
        a_units = [(rc, g) for g in range(8) for rc in range(TS // RC)]
        k = 0
        for cp in copies[2]:
            wait(cp)
        nfb = 3 * D // FB
        xp_s[...] = pltpu.bitcast(xb_ref[...], jnp.uint32)
        for c in range(nfb):
            qkv_b(c, FB)
            while k < len(a_units) and k * nfb < (c + 1) * len(a_units):
                a_unit(*a_units[k]); k += 1
        b_units = [(qi, g) for qi in range(TS // QB) for g in range(8)]
        s_next = b_qk(*b_units[0])
        for cp in copies[1] + copies[3]:
            wait(cp)
        fill = [(out_a, (c, 128)) for c in range(8)] + [(out_b, (0, c, 256)) for c in range(4)]
        for i, u in enumerate(b_units):
            s_cur = s_next
            if i + 1 < len(b_units):
                s_next = b_qk(*b_units[i + 1])
            b_rest(*u, s_cur)
            if i < 4 or i >= 8:
                pass
            j = i - 1
            if 0 <= j < 8 and j % 1 == 0:
                f, a_ = fill[j]; f(*a_)
            if i >= 10 and i < 14:
                f, a_ = fill[8 + i - 10]; f(*a_)
        for c in range(2):
            out_b(1, c, 512)

    body()


@jax.jit
def pallas_concat_heads__sliding_local_dilated__sliding_block__prompt_kernel(
    A_x: jax.Array,
    A_wqkv: jax.Array,
    A_wo: jax.Array,
    B_x: jax.Array,
    B_wqkv: jax.Array,
    B_wo: jax.Array,
):
    bf16, f32 = jnp.bfloat16, jnp.float32
    xa = A_x.reshape(S, D)
    xb = B_x.reshape(S, D)
    n_sems = 2 * (NQKV + NO)
    out = pl.pallas_call(
        _kernel,
        grid=(NB,),
        in_specs=[
            pl.BlockSpec((TS, D), lambda i: (i, 0)),
            pl.BlockSpec((TS, D), lambda i: (i, 0)),
            pl.BlockSpec(memory_space=pl.ANY),
            pl.BlockSpec(memory_space=pl.ANY),
            pl.BlockSpec(memory_space=pl.ANY),
            pl.BlockSpec(memory_space=pl.ANY),
        ],
        out_specs=pl.BlockSpec((TS, 2 * D), lambda i: (i, 0)),
        out_shape=jax.ShapeDtypeStruct((S, 2 * D), bf16),
        scratch_shapes=[
            pltpu.VMEM((D, 3 * D), bf16),
            pltpu.VMEM((D, D), bf16),
            pltpu.VMEM((D, 3 * D), bf16),
            pltpu.VMEM((D, D), bf16),
            pltpu.VMEM((TS, D), f32),
            pltpu.VMEM((8, PADA + S, 128), f32),
            pltpu.VMEM((8, PADA + S, 128), f32),
            pltpu.VMEM((TS // 2, D), jnp.uint32),
            pltpu.VMEM(((WB + S) // 2, D), jnp.uint32),
            pltpu.VMEM((D // 2, WB + S), jnp.uint32),
            pltpu.VMEM((TS // 2, D), jnp.uint32),
            pltpu.VMEM((TS // 2, D), jnp.uint32),
            pltpu.VMEM((TS // 2, D), jnp.uint32),
            pltpu.VMEM((TS // 2, D), jnp.uint32),
            pltpu.SemaphoreType.DMA((n_sems,)),
        ],
        compiler_params=pltpu.CompilerParams(
            dimension_semantics=("arbitrary",),
            vmem_limit_bytes=100 * 1024 * 1024,
        ),
    )(xa, xb, A_wqkv, A_wo, B_wqkv, B_wo)
    return out.reshape(1, S, 2 * D)
```

```python
import jax
import jax.numpy as jnp
from jax import lax
import jax.experimental.pallas as pl
import jax.experimental.pallas.tpu as pltpu

S, D, H, DH = 2048, 1024, 32, 32
TS = 256
NB = S // TS
QB = 128
WB = 256
WA, DIL = 8, 2
PADA = 16
NEG = -1e9
LOG2E = 1.4426950408889634
QSCALE = (DH ** -0.5) * LOG2E
NCHUNK = 512
NQKV = 3 * D // NCHUNK
NO = D // NCHUNK
FB = 128
ASLACK = 4


def _kernel(xa_ref, xb_ref, wqkva_hbm, woa_hbm, wqkvb_hbm, wob_hbm, out_ref,
            wqkva, woa, wqkvb, wob, qa_s, ka_s, va_s, qb_s, kb_s, vb_s, oa_s, ob_s, xp_s, xpa_s, sems):
    step = pl.program_id(0)
    f32, bf16 = jnp.float32, jnp.bfloat16

    copies = []
    sid = 0
    for src, dst, n in ((wqkva_hbm, wqkva, NQKV), (woa_hbm, woa, NO),
                        (wqkvb_hbm, wqkvb, NQKV), (wob_hbm, wob, NO)):
        lst = []
        for c in range(n):
            cs = pl.ds(c * NCHUNK, NCHUNK)
            lst.append(pltpu.make_async_copy(src.at[:, cs], dst.at[:, cs], sems.at[sid]))
            sid += 1
        copies.append(lst)

    row0 = pl.multiple_of(step * TS, TS)
    row0h = pl.multiple_of(step * (TS // 2), TS // 2)

    first = step == 0

    @pl.when(first)
    def _():
        for cp in copies[0]:
            cp.start()
        ka_s[:, pl.ds(0, PADA), :] = jnp.zeros((8, PADA, 128), f32)
        va_s[:, pl.ds(0, PADA), :] = jnp.zeros((8, PADA, 128), f32)
        kb_s[pl.ds(0, WB // 2), :] = jnp.zeros((WB // 2, D), jnp.uint32)
        vb_s[:, pl.ds(0, WB)] = jnp.zeros((D // 2, WB), jnp.uint32)
        for cp in copies[0]:
            cp.wait()
        for lst in (copies[2], copies[1], copies[3]):
            for cp in lst:
                cp.start()

    def body():
        def wait(cp):
            @pl.when(first)
            def _():
                cp.wait()

        def qkv_a(c):
            xa = pltpu.bitcast(xpa_s[...], bf16)
            r = jnp.dot(xa, wqkva[:, c * NCHUNK:(c + 1) * NCHUNK], preferred_element_type=f32)
            r = r.astype(bf16).astype(f32)
            which, col = divmod(c * NCHUNK, D)
            if which == 0:
                qa_s[:, col:col + NCHUNK] = r * QSCALE
            else:
                dst = ka_s if which == 1 else va_s
                for j in range(NCHUNK // 128):
                    dst[col // 128 + j, pl.ds(row0 + PADA, TS), :] = r[:, j * 128:(j + 1) * 128]

        et = jnp.where(lax.broadcasted_iota(jnp.int32, (16, 128), 0)
                       == lax.broadcasted_iota(jnp.int32, (16, 128), 1) // DH, 1.0, 0.0).astype(bf16)
        lane_q = lax.broadcasted_iota(jnp.int32, (QB // 2, 128), 1) // DH

        def a_logits(tt, g):
            lanes = slice(g * 128, (g + 1) * 128)
            r_loc = tt * QB
            q = qa_s[r_loc:r_loc + QB, lanes]
            base = pl.multiple_of(row0 + r_loc, QB)
            kwin = ka_s.at[g, pl.ds(base, QB + PADA), :]
            prods = [q * kwin[PADA - DIL * w:PADA - DIL * w + QB, :] for w in range(WA)]
            pr = jnp.concatenate(prods, axis=0).astype(bf16)
            lt = lax.dot_general(et, pr, (((1,), (1,)), ((), ())), preferred_element_type=f32)
            return lt[0:8]

        def a_softmax(tt, lt):
            ls = [lt[:, w * QB:(w + 1) * QB] for w in range(WA)]
            if tt == 0:
                pos = row0 + lax.broadcasted_iota(jnp.int32, (8, QB), 1)
                ls = [ls[0]] + [jnp.where(pos >= DIL * w, ls[w], NEG) for w in range(1, WA)]
            m = ls[0]
            for w in range(1, WA):
                m = jnp.maximum(m, ls[w])
            ps = [jnp.exp2(l_ - m) for l_ in ls]
            den = ps[0]
            for w in range(1, WA):
                den = den + ps[w]
            inv = pl.reciprocal(den, approx=True)
            return [p * inv for p in ps]

        def a_pv(tt, gp, pa, pb):
            r_loc = tt * QB
            base = pl.multiple_of(row0 + r_loc, QB)
            pt = pltpu.bitcast(jnp.concatenate(pa + pb, axis=0).T.astype(bf16), jnp.int32)
            for gl in range(2):
                g = 2 * gp + gl
                vwin = va_s.at[g, pl.ds(base, QB + PADA), :]
                acc = None
                for w in range(WA):
                    pe = pltpu.bitcast(jnp.take_along_axis(pt, gl * 64 + w * 8 + lane_q, axis=1), bf16).astype(f32)
                    pv = pe * vwin[PADA - DIL * w:PADA - DIL * w + QB, :]
                    acc = pv if acc is None else acc + pv
                oa_s[r_loc // 2:(r_loc + QB) // 2, g * 128:(g + 1) * 128] = pltpu.bitcast(acc.astype(bf16), jnp.uint32)

        def a_unit(tt, gp):
            pa = a_softmax(tt, a_logits(tt, 2 * gp))
            pb = a_softmax(tt, a_logits(tt, 2 * gp + 1))
            a_pv(tt, gp, pa, pb)

        def out_a(c, wd):
            r = jnp.dot(pltpu.bitcast(oa_s[...], bf16), woa[:, c * wd:(c + 1) * wd], preferred_element_type=f32)
            out_ref[:, c * wd:(c + 1) * wd] = r.astype(bf16)

        def qkv_b(c, wd):
            xb = pltpu.bitcast(xp_s[...], bf16)
            r = jnp.dot(xb, wqkvb[:, c * wd:(c + 1) * wd], preferred_element_type=f32)
            which, col = divmod(c * wd, D)
            if which == 0:
                qb_s[:, col:col + wd] = pltpu.bitcast((r * QSCALE).astype(bf16), jnp.uint32)
            elif which == 1:
                kb_s[pl.ds(row0h + WB // 2, TS // 2), col:col + wd] = pltpu.bitcast(r.astype(bf16), jnp.uint32)
            else:
                vb_s[col // 2:(col + wd) // 2, pl.ds(row0 + WB, TS)] = pltpu.bitcast(r.T.astype(bf16), jnp.uint32)

        lane_head = lax.broadcasted_iota(jnp.int32, (QB, 128), 1) // DH
        b_idx = lax.broadcasted_iota(jnp.int32, (QB, 4 * QB), 0)
        a_idx = lax.broadcasted_iota(jnp.int32, (QB, 4 * QB), 1) % QB
        causal = b_idx <= a_idx

        def b_qk(qi, g):
            lanes = slice(g * 128, (g + 1) * 128)
            r_loc = qi * QB
            r_globh = pl.multiple_of(row0h + r_loc // 2, QB // 2)
            q4 = pltpu.bitcast(qb_s[r_loc // 2:(r_loc + QB) // 2, lanes], bf16)
            qs = jnp.concatenate(
                [jnp.where(lane_head == h, q4, jnp.zeros_like(q4)) for h in range(4)], axis=0)
            k4 = pltpu.bitcast(kb_s[pl.ds(r_globh, 3 * QB // 2), lanes], bf16)
            return lax.dot_general(k4, qs, (((1,), (1,)), ((), ())), preferred_element_type=f32)

        def b_rest(qi, g, s):
            lanes = slice(g * 128, (g + 1) * 128)
            r_loc = qi * QB
            r_glob = pl.multiple_of(row0 + r_loc, QB)
            s0, s1, s2 = s[0:QB], s[QB:2 * QB], s[2 * QB:3 * QB]
            s0 = jnp.where(first, NEG, s0)
            if qi == 0:
                s1 = jnp.where(first, NEG, s1)
            s02 = jnp.where(causal, s2, s0)
            m = jnp.max(jnp.maximum(s02, s1), axis=0, keepdims=True)
            p02 = jnp.exp2(s02 - m)
            p1 = jnp.exp2(s1 - m)
            l = jnp.sum(p02 + p1, axis=0, keepdims=True)
            p0 = jnp.where(causal, 0.0, p02)
            p2 = jnp.where(causal, p02, 0.0)
            inv = pl.reciprocal(l, approx=True)
            ots = []
            for h in range(4):
                f0 = g * 128 + h * DH
                vt = pltpu.bitcast(vb_s[f0 // 2:(f0 + DH) // 2, pl.ds(r_glob, 3 * QB)], bf16)
                hs = slice(h * QB, (h + 1) * QB)
                ph = jnp.concatenate([p0[:, hs], p1[:, hs], p2[:, hs]], axis=0).astype(bf16)
                ot = jnp.dot(vt, ph, preferred_element_type=f32)
                ots.append(ot * inv[:, h * QB:(h + 1) * QB])
            o4 = jnp.concatenate(ots, axis=0).T
            ob_s[r_loc // 2:(r_loc + QB) // 2, lanes] = pltpu.bitcast(o4.astype(bf16), jnp.uint32)

        def out_b(qi, c, wd):
            r = jnp.dot(pltpu.bitcast(ob_s[qi * QB // 2:(qi + 1) * QB // 2, :], bf16),
                        wob[:, c * wd:(c + 1) * wd], preferred_element_type=f32)
            out_ref[qi * QB:(qi + 1) * QB, D + c * wd:D + (c + 1) * wd] = r.astype(bf16)

        xpa_s[...] = pltpu.bitcast(xa_ref[...], jnp.uint32)
        for c in range(NQKV):
            qkv_a(c)
        a_units = [(tt, gp) for gp in range(4) for tt in range(TS // QB)]
        k = 0
        for cp in copies[2]:
            wait(cp)
        nfb = 3 * D // FB
        xp_s[...] = pltpu.bitcast(xb_ref[...], jnp.uint32)
        for c in range(nfb):
            qkv_b(c, FB)
            while k < len(a_units) and k * (nfb - ASLACK) < (c + 1) * len(a_units):
                a_unit(*a_units[k]); k += 1
        b_units = [(qi, g) for qi in range(TS // QB) for g in range(8)]
        s_next = b_qk(*b_units[0])
        for cp in copies[1] + copies[3]:
            wait(cp)
        fill = [(out_a, (c, 128)) for c in range(8)] + [(out_b, (0, c, 128)) for c in range(8)]
        for i, u in enumerate(b_units):
            s_cur = s_next
            if i + 1 < len(b_units):
                s_next = b_qk(*b_units[i + 1])
            f, a_ = fill[i]; f(*a_)
            b_rest(*u, s_cur)
        for c in range(2):
            out_b(1, c, 512)

    body()


@jax.jit
def pallas_concat_heads__sliding_local_dilated__sliding_block__prompt_kernel(
    A_x: jax.Array,
    A_wqkv: jax.Array,
    A_wo: jax.Array,
    B_x: jax.Array,
    B_wqkv: jax.Array,
    B_wo: jax.Array,
):
    bf16, f32 = jnp.bfloat16, jnp.float32
    xa = A_x.reshape(S, D)
    xb = B_x.reshape(S, D)
    n_sems = 2 * (NQKV + NO)
    out = pl.pallas_call(
        _kernel,
        grid=(NB,),
        in_specs=[
            pl.BlockSpec((TS, D), lambda i: (i, 0)),
            pl.BlockSpec((TS, D), lambda i: (i, 0)),
            pl.BlockSpec(memory_space=pl.ANY),
            pl.BlockSpec(memory_space=pl.ANY),
            pl.BlockSpec(memory_space=pl.ANY),
            pl.BlockSpec(memory_space=pl.ANY),
        ],
        out_specs=pl.BlockSpec((TS, 2 * D), lambda i: (i, 0)),
        out_shape=jax.ShapeDtypeStruct((S, 2 * D), bf16),
        scratch_shapes=[
            pltpu.VMEM((D, 3 * D), bf16),
            pltpu.VMEM((D, D), bf16),
            pltpu.VMEM((D, 3 * D), bf16),
            pltpu.VMEM((D, D), bf16),
            pltpu.VMEM((TS, D), f32),
            pltpu.VMEM((8, PADA + S, 128), f32),
            pltpu.VMEM((8, PADA + S, 128), f32),
            pltpu.VMEM((TS // 2, D), jnp.uint32),
            pltpu.VMEM(((WB + S) // 2, D), jnp.uint32),
            pltpu.VMEM((D // 2, WB + S), jnp.uint32),
            pltpu.VMEM((TS // 2, D), jnp.uint32),
            pltpu.VMEM((TS // 2, D), jnp.uint32),
            pltpu.VMEM((TS // 2, D), jnp.uint32),
            pltpu.VMEM((TS // 2, D), jnp.uint32),
            pltpu.SemaphoreType.DMA((n_sems,)),
        ],
        compiler_params=pltpu.CompilerParams(
            dimension_semantics=("arbitrary",),
            vmem_limit_bytes=100 * 1024 * 1024,
        ),
    )(xa, xb, A_wqkv, A_wo, B_wqkv, B_wo)
    return out.reshape(1, S, 2 * D)
```
